```python
import os as _os
_os.environ.setdefault("JAX_PLATFORMS", "cpu")
import jax
import jax.numpy as jnp

def _softmax(x, axis=-1):
    return jax.nn.softmax(x, axis=axis)
def _gelu(x):
    return jax.nn.gelu(x, approximate=True)
def _silu(x):
    return jax.nn.silu(x)
def _sigmoid(x):
    return jax.nn.sigmoid(x)
def _layernorm(x, axis=-1, eps=1e-5):
    m = jnp.mean(x, axis=axis, keepdims=True)
    v = jnp.var(x, axis=axis, keepdims=True)
    return (x - m) / jnp.sqrt(v + eps)
def _scatter_add(tgt, idx, src, axis=0):
    return tgt.at[idx].add(src)
def _segment_sum(src, seg, n):
    return jax.ops.segment_sum(src, seg, n)
class _Rng:
    def __init__(self, key):
        self._k = key
    def _next(self):
        self._k, sub = jax.random.split(self._k)
        return sub
    def normal(self, shape):
        return jax.random.normal(self._next(), shape, dtype=jnp.bfloat16)
    def randint(self, lo, hi, shape):
        return jax.random.randint(self._next(), shape, lo, hi, dtype=jnp.int32)
    def uniform(self, shape, lo=0.0, hi=1.0):
        return jax.random.uniform(self._next(), shape, jnp.bfloat16, lo, hi)
    def permutation(self, n):
        return jax.random.permutation(self._next(), n)


kernel_name = 'concat_heads__gqa_block_cached__gqa_block_cached__near_ridge'

def setup_inputs():
    _rng = _Rng(jax.random.key(int.from_bytes(__import__("os").urandom(4), "little")))
    _w = (lambda a: (lambda t: t.astype(jnp.bfloat16) if jnp.issubdtype(t.dtype, jnp.floating) else t)(jnp.asarray(a)))
    def _A_setup():
        B, Sq, D = 16, 144, 448
        Hq, Hkv, Sk, Dh = 16, 8, 1024, 256
        assert Hq % Hkv == 0, (Hq, Hkv)
        return {
            "x": _w((lambda *s: _rng.normal(s) * 0.8)(B, Sq, D)),
            "k_cache": _w((lambda *s: _rng.normal(s) * 0.8)(B, Hkv, Sk, Dh)),
            "v_cache": _w((lambda *s: _rng.normal(s) * 0.05)(B, Hkv, Sk, Dh)),
            "wq": _w((lambda *s: _rng.normal(s) * 0.8)(D, Hq * Dh) * (D ** -0.5)),
            "wo": _w((lambda *s: _rng.normal(s) * 0.05)(Hq * Dh, D) * ((Hq * Dh) ** -0.5)),
        }
    _A_in = _A_setup()

    def _B_setup():
        B, Sq, D = 16, 144, 448
        Hq, Hkv, Sk, Dh = 16, 8, 1024, 256
        assert Hq % Hkv == 0, (Hq, Hkv)
        return {
            "x": _w((lambda *s: _rng.normal(s) * 0.8)(B, Sq, D)),
            "k_cache": _w((lambda *s: _rng.normal(s) * 0.8)(B, Hkv, Sk, Dh)),
            "v_cache": _w((lambda *s: _rng.normal(s) * 0.05)(B, Hkv, Sk, Dh)),
            "wq": _w((lambda *s: _rng.normal(s) * 0.8)(D, Hq * Dh) * (D ** -0.5)),
            "wo": _w((lambda *s: _rng.normal(s) * 0.05)(Hq * Dh, D) * ((Hq * Dh) ** -0.5)),
        }
    _B_in = _B_setup()

    return {
        "A_x": _A_in["x"],
        "A_k_cache": _A_in["k_cache"],
        "A_v_cache": _A_in["v_cache"],
        "A_wq": _A_in["wq"],
        "A_wo": _A_in["wo"],
        "B_x": _B_in["x"],
        "B_k_cache": _B_in["k_cache"],
        "B_v_cache": _B_in["v_cache"],
        "B_wq": _B_in["wq"],
        "B_wo": _B_in["wo"],
    }

def reference(A_x, A_k_cache, A_v_cache, A_wq, A_wo, B_x, B_k_cache, B_v_cache, B_wq, B_wo):
    def _A_ref(x, k_cache, v_cache, wq, wo):
        B, Sq, D = x.shape
        Hq, Dh = 16, 256
        Hkv = k_cache.shape[1]
        rep = Hq // Hkv
        q = (lambda x, *d: x.transpose(*d))((x @ wq).reshape(B, Sq, Hq, Dh), 0, 2, 1, 3)
        k = jnp.repeat(k_cache, rep, axis=1)
        v = jnp.repeat(v_cache, rep, axis=1)
        scores = jnp.einsum("bhqd,bhkd->bhqk", q, k) * (Dh ** -0.5)
        p = _softmax(scores, axis=-1)
        o = jnp.einsum("bhqk,bhkd->bhqd", p, v)
        return (lambda x, *d: x.transpose(*d))(o, 0, 2, 1, 3).reshape(B, Sq, Hq * Dh) @ wo

    def _B_ref(x, k_cache, v_cache, wq, wo):
        B, Sq, D = x.shape
        Hq, Dh = 16, 256
        Hkv = k_cache.shape[1]
        rep = Hq // Hkv
        q = (lambda x, *d: x.transpose(*d))((x @ wq).reshape(B, Sq, Hq, Dh), 0, 2, 1, 3)
        k = jnp.repeat(k_cache, rep, axis=1)
        v = jnp.repeat(v_cache, rep, axis=1)
        scores = jnp.einsum("bhqd,bhkd->bhqk", q, k) * (Dh ** -0.5)
        p = _softmax(scores, axis=-1)
        o = jnp.einsum("bhqk,bhkd->bhqd", p, v)
        return (lambda x, *d: x.transpose(*d))(o, 0, 2, 1, 3).reshape(B, Sq, Hq * Dh) @ wo

    a = _A_ref(A_x, A_k_cache, A_v_cache, A_wq, A_wo)
    b = _B_ref(B_x, B_k_cache, B_v_cache, B_wq, B_wo)
    return jnp.concatenate([a, b], axis=-1)
```

```python
import jax
import jax.numpy as jnp
import numpy as np
from jax import lax
import jax.experimental.pallas as pl
import jax.experimental.pallas.tpu as pltpu

B, SQ, D = 16, 144, 448
HKV, SK, DH = 8, 1024, 256
R = B * SQ
RH = R // 2
HD = 2 * DH
M2 = 2 * SQ
CH = 256
NCH = SK // CH

G = 8
G0 = 2
NG = B // G
XC = 576
NX = R // XC
QC = 576
OC = 384
FC = 384
NF = R // FC

Q0 = 0
O0 = 4 * RH
P0 = 8 * RH
L0 = P0 + 2 * NCH * SQ
WROWS = L0 + 2 * M2

QSCALE = float(np.log2(np.e) / np.sqrt(DH))
NT_DIMS = (((1,), (1,)), ((), ()))
F32, BF16 = jnp.float32, jnp.bfloat16


def _aligned(i, m):
    return i if isinstance(i, int) else pl.multiple_of(i, m)


def _pack(v):
    return pltpu.bitcast(v, F32)


def _unpack(v):
    return pltpu.bitcast(v, BF16)


def _kernel(xa, ka, va, wqa, woa, xb, kb, vb, wqb, wob, out,
            x_v, wq_v, wo_v, w, acc, kv_v, out_v,
            sem_x, sem_w, sem_kv, sem_kv0, sem_o, sem_b):
    xs, wqs, wos = (xa, xb), (wqa, wqb), (woa, wob)
    kvs = (ka, va, kb, vb)

    def x_copy(br, i):
        rows = pl.ds(_aligned(i * XC, XC), XC)
        return pltpu.make_async_copy(
            xs[br].at[rows], x_v.at[br, rows], sem_x.at[br * NX + i])

    def wq_copy(br, h):
        cols = pl.ds(_aligned(h * HD, HD), HD)
        return pltpu.make_async_copy(
            wqs[br].at[:, cols], wq_v.at[br], sem_w.at[br])

    def wo_copy(br, h):
        cols = pl.ds(_aligned(h * HD, HD), HD)
        return pltpu.make_async_copy(
            wos[br].at[:, cols], wo_v.at[br], sem_w.at[2 + br])

    def kv0_copy(i, t):
        bs = pl.ds(t * G0, G0)
        return pltpu.make_async_copy(
            kvs[i].at[bs, 0], kv_v.at[i, bs], sem_kv0.at[t * 4 + i])

    def kv_copy(i, h, g):
        bs = pl.ds(g * G, G)
        return pltpu.make_async_copy(
            kvs[i].at[bs, h], kv_v.at[i, bs], sem_kv.at[g * 4 + i])

    def out_copy(i):
        rows = pl.ds(_aligned(i * FC, FC), FC)
        return pltpu.make_async_copy(out_v.at[rows], out.at[rows], sem_o.at[i])

    def keep_dma_order():
        pl.semaphore_signal(sem_b, 1)
        pl.semaphore_wait(sem_b, 1)

    def prefetch(h, g):
        for i in range(4):
            kv_copy(i, h, g).start()

    def wrows(base, br, hh, r0, n):
        return pl.ds(_aligned(base + (br * 2 + hh) * RH + r0 // 2, 8), n // 2)

    def q_proj(br, r0, n):
        x = x_v[br, pl.ds(_aligned(r0, 16), n), :]
        q = jnp.dot(x, wq_v[br], preferred_element_type=F32)
        q = (q * QSCALE).astype(BF16)
        for hh in range(2):
            w[wrows(Q0, br, hh, r0, n), :] = _pack(q[:, hh * DH:(hh + 1) * DH])

    def o_proj_t(br, r0, n):
        o = jnp.concatenate(
            [_unpack(w[wrows(O0, br, hh, r0, n), :]) for hh in range(2)], axis=1)
        return lax.dot_general(wo_v[br], o, NT_DIMS, preferred_element_type=F32)

    def attention(b0, nb):
        units = [(br, j) for j in range(nb) for br in range(2)]

        def l_rows(n):
            return pl.ds(L0 + (n % 2) * M2, M2)

        def finish(n, o):
            br, j = units[n]
            l = jnp.sum(w[l_rows(n), 0:128], axis=1, keepdims=True)
            r = (o * (1.0 / l)).astype(BF16)
            r0 = (b0 + j) * SQ
            w[wrows(O0, br, 0, r0, SQ), :] = _pack(r[:SQ])
            w[wrows(O0, br, 1, r0, SQ), :] = _pack(r[SQ:])

        pending = None
        for n, (br, j) in enumerate(units):
            r0 = (b0 + j) * SQ
            s = []
            for c in range(NCH):
                if pending is not None and c == 1:
                    finish(*pending)
                q = jnp.concatenate(
                    [_unpack(w[wrows(Q0, br, hh, r0, SQ), :]) for hh in range(2)],
                    axis=0)
                k = kv_v[2 * br, b0 + j, pl.ds(c * CH, CH), :]
                s.append(lax.dot_general(q, k, NT_DIMS, preferred_element_type=F32))
            m = jnp.max(jnp.concatenate(s, axis=1), axis=1, keepdims=True)
            o = None
            for c in range(NCH):
                p = jnp.exp2(s[c] - m)
                ps = p[:, :128] + p[:, 128:]
                w[l_rows(n), 0:128] = ps if c == 0 else w[l_rows(n), 0:128] + ps
                p_rows = pl.ds(P0 + ((n % 2) * NCH + c) * SQ, SQ)
                w[p_rows, :] = _pack(p.astype(BF16))
                v = kv_v[2 * br + 1, b0 + j, pl.ds(c * CH, CH), :]
                d = jnp.dot(_unpack(w[p_rows, :]), v, preferred_element_type=F32)
                o = d if c == 0 else o + d
            pending = (n, o)
        finish(*pending)

    for br in range(2):
        wq_copy(br, 0).start()
        for i in range(NX):
            x_copy(br, i).start()
            keep_dma_order()
    for t in range(B // G0):
        for i in range(4):
            kv0_copy(i, t).start()
        keep_dma_order()
    acc[...] = jnp.zeros(acc.shape, F32)

    def first_q_proj(t, carry):
        i = t % NX
        for br in range(2):
            @pl.when(t // NX == br)
            def _():
                @pl.when(i == 0)
                def _():
                    wq_copy(br, 0).wait()
                x_copy(br, i).wait()
        q_proj(t // NX, i * XC, XC)
        return carry

    lax.fori_loop(0, 2 * NX, first_q_proj, 0)

    def head(h, carry):
        more = h < HKV - 1
        for br in range(2):
            wo_copy(br, h).start()

        @pl.when(more)
        def _():
            for br in range(2):
                wq_copy(br, h + 1).start()

        @pl.when(h == 0)
        def _():
            per = G // G0

            def block(t, c):
                for i in range(4):
                    kv0_copy(i, t).wait()
                attention(t * G0, G0)
                pl.when(t % per == per - 1)(lambda: prefetch(1, t // per))
                return c

            lax.fori_loop(0, B // G0, block, 0)

        @pl.when(h > 0)
        def _():
            def block(g, c):
                for i in range(4):
                    kv_copy(i, h, g).wait()
                attention(g * G, G)
                pl.when(more)(lambda: prefetch(h + 1, g))
                return c

            lax.fori_loop(0, NG, block, 0)

        for br in range(2):
            wo_copy(br, h).wait()

        @pl.when(more)
        def _():
            for br in range(2):
                wq_copy(br, h + 1).wait()

            def project(br, c):
                rows = pl.ds(pl.multiple_of(br * D, D), D)
                for i in range(R // OC):
                    acc[rows, pl.ds(i * OC, OC)] += o_proj_t(br, i * OC, OC)
                for i in range(R // QC):
                    q_proj(br, i * QC, QC)
                return c

            lax.fori_loop(0, 2, project, 0)

        return carry

    lax.fori_loop(0, HKV, head, 0)

    def final(i, carry):
        for k in range(FC // 128):
            r0 = pl.multiple_of(i * FC + k * 128, 128)
            t = jnp.concatenate(
                [acc[br * D:(br + 1) * D, pl.ds(r0, 128)] + o_proj_t(br, r0, 128)
                 for br in range(2)], axis=0)
            out_v[pl.ds(r0, 128), :] = t.T.astype(BF16)
        out_copy(i).start()
        return carry

    lax.fori_loop(0, NF, final, 0)
    for i in range(NF):
        out_copy(i).wait()


@jax.jit
def pallas_concat_heads__gqa_block_cached__gqa_block_cached__near_ridge_kernel(
    A_x: jax.Array,
    A_k_cache: jax.Array,
    A_v_cache: jax.Array,
    A_wq: jax.Array,
    A_wo: jax.Array,
    B_x: jax.Array,
    B_k_cache: jax.Array,
    B_v_cache: jax.Array,
    B_wq: jax.Array,
    B_wo: jax.Array,
):
    hbm = pl.BlockSpec(memory_space=pltpu.HBM)
    out = pl.pallas_call(
        _kernel,
        in_specs=[hbm] * 10,
        out_specs=hbm,
        out_shape=jax.ShapeDtypeStruct((R, 2 * D), BF16),
        scratch_shapes=[
            pltpu.VMEM((2, R, D), BF16),
            pltpu.VMEM((2, D, HD), BF16),
            pltpu.VMEM((2, D, HD), BF16),
            pltpu.VMEM((WROWS, DH), F32),
            pltpu.VMEM((2 * D, R), F32),
            pltpu.VMEM((4, B, SK, DH), BF16),
            pltpu.VMEM((R, 2 * D), BF16),
            pltpu.SemaphoreType.DMA((2 * NX,)),
            pltpu.SemaphoreType.DMA((4,)),
            pltpu.SemaphoreType.DMA((NG * 4,)),
            pltpu.SemaphoreType.DMA((B // G0 * 4,)),
            pltpu.SemaphoreType.DMA((NF,)),
            pltpu.SemaphoreType.REGULAR,
        ],
        compiler_params=pltpu.CompilerParams(vmem_limit_bytes=120 * 2**20),
    )(A_x.reshape(R, D), A_k_cache, A_v_cache, A_wq, A_wo.T,
      B_x.reshape(R, D), B_k_cache, B_v_cache, B_wq, B_wo.T)
    return out.reshape(B, SQ, 2 * D)
```

```python
import functools

import jax
import jax.numpy as jnp
import numpy as np
from jax import lax
import jax.experimental.pallas as pl
import jax.experimental.pallas.tpu as pltpu

B, SQ, D = 16, 144, 448
HKV, SK, DH = 8, 1024, 256
R = B * SQ
RH = R // 2
HD = 2 * DH
M2 = 2 * SQ
CH = 256
NCH = SK // CH

G = 8
G0 = 2
NG = B // G
XC = 576
NX = R // XC
QC = 576
OC = 384
FIRST = (0, 1, 3, 6, 2 * NX)
FINAL = ((4, 512), (2, 128))

Q0 = 0
O0 = 4 * RH
P0 = 8 * RH
L0 = P0 + 2 * NCH * SQ
WROWS = L0 + 2 * M2

QSCALE = float(np.log2(np.e) / np.sqrt(DH))
NT_DIMS = (((1,), (1,)), ((), ()))
F32, BF16 = jnp.float32, jnp.bfloat16


def _aligned(i, m):
    return i if isinstance(i, int) else pl.multiple_of(i, m)


def _pack(v):
    return pltpu.bitcast(v, F32)


def _unpack(v):
    return pltpu.bitcast(v, BF16)


def _kernel(xa, ka, va, wqa, woa, xb, kb, vb, wqb, wob, out,
            x_v, wq_v, wo_v, w, acc, kv_v, out_v,
            sem, sem_kv0, sem_order):
    xs, wqs, wos = (xa, xb), (wqa, wqb), (woa, wob)
    kvs = (ka, va, kb, vb)

    def wq_copy(br, h, k=2):
        cols = pl.ds(_aligned(h * HD, HD), HD)
        return pltpu.make_async_copy(wqs[br].at[:, cols], wq_v.at[br], sem.at[k])

    def wo_copy(br, h):
        cols = pl.ds(_aligned(h * HD, HD), HD)
        return pltpu.make_async_copy(wos[br].at[:, cols], wo_v.at[br], sem.at[3])

    def first_copies(k):
        copies = []
        for t in range(FIRST[k], FIRST[k + 1]):
            br, rows = t // NX, pl.ds((t % NX) * XC, XC)
            if t % NX == 0:
                copies.append(wq_copy(br, 0, k))
            copies.append(pltpu.make_async_copy(
                xs[br].at[rows], x_v.at[br, rows], sem.at[k]))
        return copies

    def kv0_copy(i, t):
        bs = pl.ds(t * G0, G0)
        return pltpu.make_async_copy(kvs[i].at[bs, 0], kv_v.at[i, bs], sem_kv0.at[t])

    def kv_copy(i, h, g):
        bs = pl.ds(g * G, G)
        return pltpu.make_async_copy(kvs[i].at[bs, h], kv_v.at[i, bs], sem.at[g])

    def out_copy(r0, n):
        rows = pl.ds(_aligned(r0, 128), n)
        return pltpu.make_async_copy(out_v.at[rows], out.at[rows], sem.at[0])

    def keep_dma_order():
        pl.semaphore_signal(sem_order, 1)
        pl.semaphore_wait(sem_order, 1)

    def prefetch(h, g):
        for i in range(4):
            kv_copy(i, h, g).start()

    def wrows(base, br, hh, r0, n):
        return pl.ds(_aligned(base + (br * 2 + hh) * RH + r0 // 2, 8), n // 2)

    def q_proj(br, r0, n):
        x = x_v[br, pl.ds(_aligned(r0, 16), n), :]
        q = jnp.dot(x, wq_v[br], preferred_element_type=F32)
        q = (q * QSCALE).astype(BF16)
        for hh in range(2):
            w[wrows(Q0, br, hh, r0, n), :] = _pack(q[:, hh * DH:(hh + 1) * DH])

    def o_proj_t(br, r0, n):
        o = jnp.concatenate(
            [_unpack(w[wrows(O0, br, hh, r0, n), :]) for hh in range(2)], axis=1)
        return lax.dot_general(wo_v[br], o, NT_DIMS, preferred_element_type=F32)

    def attention(b0, nb):
        units = [(br, j) for j in range(nb) for br in range(2)]

        def l_rows(n):
            return pl.ds(L0 + (n % 2) * M2, M2)

        def finish(n, o):
            br, j = units[n]
            l = jnp.sum(w[l_rows(n), 0:128], axis=1, keepdims=True)
            r = (o * (1.0 / l)).astype(BF16)
            r0 = (b0 + j) * SQ
            w[wrows(O0, br, 0, r0, SQ), :] = _pack(r[:SQ])
            w[wrows(O0, br, 1, r0, SQ), :] = _pack(r[SQ:])

        pending = None
        for n, (br, j) in enumerate(units):
            r0 = (b0 + j) * SQ
            s = []
            for c in range(NCH):
                if pending is not None and c == NCH - 1:
                    finish(*pending)
                q = jnp.concatenate(
                    [_unpack(w[wrows(Q0, br, hh, r0, SQ), :]) for hh in range(2)],
                    axis=0)
                k = kv_v[2 * br, b0 + j, pl.ds(c * CH, CH), :]
                s.append(lax.dot_general(q, k, NT_DIMS, preferred_element_type=F32))
            m = None
            for sc in s:
                mc = jnp.maximum(sc[:, :128], sc[:, 128:])
                m = mc if m is None else jnp.maximum(mc, m)
            m = jnp.max(m, axis=1, keepdims=True)
            o = l = None
            for c in reversed(range(NCH)):
                p = jnp.exp2(s[c] - m)
                p_rows = pl.ds(P0 + ((n % 2) * NCH + c) * SQ, SQ)
                w[p_rows, :] = _pack(p.astype(BF16))
                l = p[:, :128] + p[:, 128:] if l is None else l + p[:, :128] + p[:, 128:]
                if c == 0:
                    w[l_rows(n), 0:128] = l
                v = kv_v[2 * br + 1, b0 + j, pl.ds(c * CH, CH), :]
                d = jnp.dot(_unpack(w[p_rows, :]), v, preferred_element_type=F32)
                o = d if o is None else d + o
            pending = (n, o)
        finish(*pending)

    for k in range(len(FIRST) - 1):
        for copy in first_copies(k):
            copy.start()
        keep_dma_order()
    for t in range(B // G0):
        for i in range(4):
            kv0_copy(i, t).start()
        keep_dma_order()

    def first_q_proj(t, carry):
        for k in range(len(FIRST) - 1):
            @pl.when(t == FIRST[k])
            def _():
                for copy in first_copies(k):
                    copy.wait()
        q_proj(t // NX, (t % NX) * XC, XC)
        return carry

    lax.fori_loop(0, 2 * NX, first_q_proj, 0)

    def head(h, carry):
        more = h < HKV - 1
        for br in range(2):
            wo_copy(br, h).start()

        @pl.when(more)
        def _():
            for br in range(2):
                wq_copy(br, h + 1).start()

        @pl.when(h == 0)
        def _():
            def group(g, c):
                def block(u, c):
                    t = g * (G // G0) + u
                    for i in range(4):
                        kv0_copy(i, t).wait()
                    attention(t * G0, G0)
                    return c

                lax.fori_loop(0, G // G0, block, 0)
                prefetch(1, g)
                return c

            lax.fori_loop(0, NG, group, 0)

        @pl.when(h > 0)
        def _():
            def block(g, c):
                for i in range(4):
                    kv_copy(i, h, g).wait()
                attention(g * G, G)
                pl.when(more)(lambda: prefetch(h + 1, g))
                return c

            lax.fori_loop(0, NG, block, 0)

        for br in range(2):
            wo_copy(br, h).wait()

        @pl.when(more)
        def _():
            for br in range(2):
                wq_copy(br, h + 1).wait()

            def project(br, c):
                rows = pl.ds(pl.multiple_of(br * D, D), D)
                for i in range(R // OC):
                    cols = pl.ds(i * OC, OC)
                    prev = jnp.where(h > 0, acc[rows, cols], 0.0)
                    acc[rows, cols] = o_proj_t(br, i * OC, OC) + prev
                for i in range(R // QC):
                    q_proj(br, i * QC, QC)
                return c

            lax.fori_loop(0, 2, project, 0)

        return carry

    lax.fori_loop(0, HKV, head, 0)

    def final(base, n, i, carry):
        for k in range(n // 128):
            r0 = pl.multiple_of(base + i * n + k * 128, 128)
            t = jnp.concatenate(
                [o_proj_t(br, r0, 128) + acc[br * D:(br + 1) * D, pl.ds(r0, 128)]
                 for br in range(2)], axis=0)
            out_v[pl.ds(r0, 128), :] = t.T.astype(BF16)
        out_copy(base + i * n, n).start()
        return carry

    base, written = 0, []
    for steps, n in FINAL:
        lax.fori_loop(0, steps, functools.partial(final, base, n), 0)
        written += [(base + i * n, n) for i in range(steps)]
        base += steps * n
    assert base == R
    for r0, n in written:
        out_copy(r0, n).wait()


@jax.jit
def pallas_concat_heads__gqa_block_cached__gqa_block_cached__near_ridge_kernel(
    A_x: jax.Array,
    A_k_cache: jax.Array,
    A_v_cache: jax.Array,
    A_wq: jax.Array,
    A_wo: jax.Array,
    B_x: jax.Array,
    B_k_cache: jax.Array,
    B_v_cache: jax.Array,
    B_wq: jax.Array,
    B_wo: jax.Array,
):
    hbm = pl.BlockSpec(memory_space=pltpu.HBM)
    out = pl.pallas_call(
        _kernel,
        in_specs=[hbm] * 10,
        out_specs=hbm,
        out_shape=jax.ShapeDtypeStruct((R, 2 * D), BF16),
        scratch_shapes=[
            pltpu.VMEM((2, R, D), BF16),
            pltpu.VMEM((2, D, HD), BF16),
            pltpu.VMEM((2, D, HD), BF16),
            pltpu.VMEM((WROWS, DH), F32),
            pltpu.VMEM((2 * D, R), F32),
            pltpu.VMEM((4, B, SK, DH), BF16),
            pltpu.VMEM((R, 2 * D), BF16),
            pltpu.SemaphoreType.DMA((4,)),
            pltpu.SemaphoreType.DMA((B // G0,)),
            pltpu.SemaphoreType.REGULAR,
        ],
        compiler_params=pltpu.CompilerParams(vmem_limit_bytes=120 * 2**20),
    )(A_x.reshape(R, D), A_k_cache, A_v_cache, A_wq, A_wo.T,
      B_x.reshape(R, D), B_k_cache, B_v_cache, B_wq, B_wo.T)
    return out.reshape(B, SQ, 2 * D)
```
